```python
import os as _os
_os.environ.setdefault("JAX_PLATFORMS", "cpu")
import jax
import jax.numpy as jnp

def _softmax(x, axis=-1):
    return jax.nn.softmax(x, axis=axis)
def _gelu(x):
    return jax.nn.gelu(x, approximate=True)
def _silu(x):
    return jax.nn.silu(x)
def _sigmoid(x):
    return jax.nn.sigmoid(x)
def _layernorm(x, axis=-1, eps=1e-5):
    m = jnp.mean(x, axis=axis, keepdims=True)
    v = jnp.var(x, axis=axis, keepdims=True)
    return (x - m) / jnp.sqrt(v + eps)
def _scatter_add(tgt, idx, src, axis=0):
    return tgt.at[idx].add(src)
def _segment_sum(src, seg, n):
    return jax.ops.segment_sum(src, seg, n)
class _Rng:
    def __init__(self, key):
        self._k = key
    def _next(self):
        self._k, sub = jax.random.split(self._k)
        return sub
    def normal(self, shape):
        return jax.random.normal(self._next(), shape, dtype=jnp.bfloat16)
    def randint(self, lo, hi, shape):
        return jax.random.randint(self._next(), shape, lo, hi, dtype=jnp.int32)
    def uniform(self, shape, lo=0.0, hi=1.0):
        return jax.random.uniform(self._next(), shape, jnp.bfloat16, lo, hi)
    def permutation(self, n):
        return jax.random.permutation(self._next(), n)


kernel_name = 'standalone__mha_softmax__near_ridge'

def setup_inputs():
    _rng = _Rng(jax.random.key(int.from_bytes(__import__("os").urandom(4), "little")))
    _w = (lambda a: (lambda t: t.astype(jnp.bfloat16) if jnp.issubdtype(t.dtype, jnp.floating) else t)(jnp.asarray(a)))
    B, H, Sq, Sk, D = 8, 32, 304, 2048, 128
    return {
        "q": _w((lambda *s: _rng.normal(s) * 0.4)(B, H, Sq, D)),
        "k": _w((lambda *s: _rng.normal(s) * 0.4)(B, H, Sk, D)),
        "v": _w((lambda *s: _rng.normal(s) * 0.05)(B, H, Sk, D)),
    }

def reference(q, k, v):
    scale = q.shape[-1] ** -0.5
    scores = jnp.einsum("bhqd,bhkd->bhqk", q, k) * scale
    p = _softmax(scores, axis=-1)
    return jnp.einsum("bhqk,bhkd->bhqd", p, v)
```

```python
import functools

import jax
import jax.numpy as jnp
from jax import lax
import jax.experimental.pallas as pl
import jax.experimental.pallas.tpu as pltpu


def _attn_kernel(q_ref, k_ref, v_ref, o_ref, *, scale):
    q = q_ref[...]
    k = k_ref[...]
    v = v_ref[...]
    s = lax.dot_general(q, k, (((1,), (1,)), ((), ())),
                        preferred_element_type=jnp.float32)
    s = s * scale
    m = jnp.max(s, axis=-1, keepdims=True)
    p = jnp.exp(s - m)
    l = jnp.sum(p, axis=-1, keepdims=True)
    o = jnp.dot(p.astype(v.dtype), v, preferred_element_type=jnp.float32)
    o_ref[...] = (o / l).astype(o_ref.dtype)


@jax.jit
def pallas_standalone__mha_softmax__near_ridge_kernel(
    q: jax.Array,
    k: jax.Array,
    v: jax.Array,
):
    B, H, Sq, D = q.shape
    Sk = k.shape[2]
    scale = float(D) ** -0.5
    q3 = q.reshape(B * H, Sq, D)
    k3 = k.reshape(B * H, Sk, D)
    v3 = v.reshape(B * H, Sk, D)

    out = pl.pallas_call(
        functools.partial(_attn_kernel, scale=scale),
        grid=(B * H,),
        in_specs=[
            pl.BlockSpec((None, Sq, D), lambda i: (i, 0, 0)),
            pl.BlockSpec((None, Sk, D), lambda i: (i, 0, 0)),
            pl.BlockSpec((None, Sk, D), lambda i: (i, 0, 0)),
        ],
        out_specs=pl.BlockSpec((None, Sq, D), lambda i: (i, 0, 0)),
        out_shape=jax.ShapeDtypeStruct((B * H, Sq, D), q.dtype),
        compiler_params=pltpu.CompilerParams(
            dimension_semantics=("parallel",),
            vmem_limit_bytes=64 * 1024 * 1024,
        ),
    )(q3, k3, v3)
    return out.reshape(B, H, Sq, D)
```

```python
import functools
import math

import jax
import jax.numpy as jnp
from jax import lax
import jax.experimental.pallas as pl
import jax.experimental.pallas.tpu as pltpu

HEADS_PER_STEP = 8
KV_CHUNK = 512
_LANES = 128
_CONTRACT_LAST = (((1,), (1,)), ((), ()))


def _fold_lane_tiles(x, op):
    acc = x[:, :_LANES]
    for t in range(1, x.shape[1] // _LANES):
        acc = op(acc, x[:, t * _LANES:(t + 1) * _LANES])
    return acc


def _order_after(x, deps, zero):
    d = lax.bitcast_convert_type(deps[0], jnp.int32)
    for dep in deps[1:]:
        d = d | lax.bitcast_convert_type(dep, jnp.int32)
    xi = lax.bitcast_convert_type(x, jnp.int32)
    return lax.bitcast_convert_type(xi | (d & zero), jnp.float32)


def _reciprocal_of_row_sum(l):
    r = pl.reciprocal(l, approx=True)
    r = r * (2.0 - l * r)
    r = r * (2.0 - l * r)
    return r


def _attention_kernel(q_ref, k_ref, v_ref, o_ref, *, exp2_scale):
    heads, sq, _ = q_ref.shape
    sk = k_ref.shape[1]
    n_chunks = sk // KV_CHUNK
    zero = jnp.full((sq, _LANES), pl.program_id(0) >> 30, jnp.int32)

    finished = []
    for h in range(heads):
        q = q_ref[h]
        m_run = l_run = acc = None
        for j in range(n_chunks):
            k = k_ref[h, pl.ds(j * KV_CHUNK, KV_CHUNK), :]
            v = v_ref[h, pl.ds(j * KV_CHUNK, KV_CHUNK), :]
            s = lax.dot_general(q, k, _CONTRACT_LAST,
                                preferred_element_type=jnp.float32)
            m_chunk = jnp.max(s, axis=-1, keepdims=True)
            m_new = m_chunk if j == 0 else jnp.maximum(m_run, m_chunk)
            p = jnp.exp2((s - m_new) * exp2_scale)
            l_chunk = _fold_lane_tiles(p, jnp.add)
            deps = [l_chunk] + (finished if j == 0 else [])
            if j == 0:
                finished = []
            p = jnp.concatenate(
                [_order_after(p[:, :_LANES], deps, zero), p[:, _LANES:]], axis=1)
            pv = jnp.dot(p.astype(v.dtype), v, preferred_element_type=jnp.float32)
            if j == 0:
                l_run, acc = l_chunk, pv
            else:
                alpha = jnp.exp2((m_run - m_new) * exp2_scale)
                l_run = alpha * l_run + l_chunk
                acc = alpha * acc + pv
            m_run = m_new
        l_row = jnp.sum(l_run, axis=-1, keepdims=True)
        out = acc * _reciprocal_of_row_sum(l_row)
        finished = [out]
        o_ref[h] = out.astype(o_ref.dtype)


@jax.jit
def pallas_standalone__mha_softmax__near_ridge_kernel(
    q: jax.Array,
    k: jax.Array,
    v: jax.Array,
):
    B, H, Sq, D = q.shape
    Sk = k.shape[2]
    n_heads = B * H
    hb = HEADS_PER_STEP
    assert n_heads % hb == 0 and Sk % KV_CHUNK == 0
    exp2_scale = float(D) ** -0.5 * math.log2(math.e)

    q3 = q.reshape(n_heads, Sq, D)
    k3 = k.reshape(n_heads, Sk, D)
    v3 = v.reshape(n_heads, Sk, D)

    out = pl.pallas_call(
        functools.partial(_attention_kernel, exp2_scale=exp2_scale),
        grid=(n_heads // hb,),
        in_specs=[
            pl.BlockSpec((hb, Sq, D), lambda i: (i, 0, 0)),
            pl.BlockSpec((hb, Sk, D), lambda i: (i, 0, 0)),
            pl.BlockSpec((hb, Sk, D), lambda i: (i, 0, 0)),
        ],
        out_specs=pl.BlockSpec((hb, Sq, D), lambda i: (i, 0, 0)),
        out_shape=jax.ShapeDtypeStruct((n_heads, Sq, D), q.dtype),
        compiler_params=pltpu.CompilerParams(
            dimension_semantics=("arbitrary",),
            vmem_limit_bytes=96 * 1024 * 1024,
        ),
    )(q3, k3, v3)
    return out.reshape(B, H, Sq, D)
```
